```python
import os as _os
_os.environ.setdefault("JAX_PLATFORMS", "cpu")
import jax
import jax.numpy as jnp

def _softmax(x, axis=-1):
    return jax.nn.softmax(x, axis=axis)
def _gelu(x):
    return jax.nn.gelu(x, approximate=True)
def _silu(x):
    return jax.nn.silu(x)
def _sigmoid(x):
    return jax.nn.sigmoid(x)
def _layernorm(x, axis=-1, eps=1e-5):
    m = jnp.mean(x, axis=axis, keepdims=True)
    v = jnp.var(x, axis=axis, keepdims=True)
    return (x - m) / jnp.sqrt(v + eps)
def _scatter_add(tgt, idx, src, axis=0):
    return tgt.at[idx].add(src)
def _segment_sum(src, seg, n):
    return jax.ops.segment_sum(src, seg, n)
class _Rng:
    def __init__(self, key):
        self._k = key
    def _next(self):
        self._k, sub = jax.random.split(self._k)
        return sub
    def normal(self, shape):
        return jax.random.normal(self._next(), shape, dtype=jnp.bfloat16)
    def randint(self, lo, hi, shape):
        return jax.random.randint(self._next(), shape, lo, hi, dtype=jnp.int32)
    def uniform(self, shape, lo=0.0, hi=1.0):
        return jax.random.uniform(self._next(), shape, jnp.bfloat16, lo, hi)
    def permutation(self, n):
        return jax.random.permutation(self._next(), n)


kernel_name = 'sequential_preLN__compressed_kv_cla__dense_activation_mish__decode'

def setup_inputs():
    _rng = _Rng(jax.random.key(int.from_bytes(__import__("os").urandom(4), "little")))
    _w = (lambda a: (lambda t: t.astype(jnp.bfloat16) if jnp.issubdtype(t.dtype, jnp.floating) else t)(jnp.asarray(a)))
    def _A_setup():
        B, H, Sq, Sk, D, M = 2, 32, 1, 8192, 128, 512
        Dc = 4 * D
        return {
            "x": _w((lambda *s: _rng.normal(s) * 0.05)(B, Sq, M)),
            "c_kv": _w((lambda *s: _rng.normal(s) * 0.8)(B, Sk, Dc)),
            "w_q": _w((lambda *s: _rng.normal(s) * 0.8)(M, H, D) * (M ** -0.5)),
            "w_uk": _w((lambda *s: _rng.normal(s) * 0.8)(Dc, H, D) * (Dc ** -0.5)),
            "w_uv": _w((lambda *s: _rng.normal(s) * 0.8)(Dc, H, D) * (Dc ** -0.5)),
            "w_o": _w((lambda *s: _rng.normal(s) * 0.8)(H, D, M) * ((H * D) ** -0.5)),
        }
    _A_in = _A_setup()

    def _B_setup():
        B, S, D, F = 2, 1, 512, 1792
        return {
            "x": _w((lambda *s: _rng.normal(s) * 0.05)(B, S, D)),
            "w1": _w((lambda *s: _rng.normal(s) * 0.4)(D, F) * (D ** -0.5)),
            "b1": _w((lambda *s: _rng.normal(s) * 0.05)(F)),
            "w2": _w((lambda *s: _rng.normal(s) * 0.05)(F, D) * (F ** -0.5)),
        }
    _B_in = _B_setup()

    return {
        "A_x": _A_in["x"],
        "A_c_kv": _A_in["c_kv"],
        "A_w_q": _A_in["w_q"],
        "A_w_uk": _A_in["w_uk"],
        "A_w_uv": _A_in["w_uv"],
        "A_w_o": _A_in["w_o"],
        "B_x": _B_in["x"],
        "B_w1": _B_in["w1"],
        "B_b1": _B_in["b1"],
        "B_w2": _B_in["w2"],
    }

def reference(A_x, A_c_kv, A_w_q, A_w_uk, A_w_uv, A_w_o, B_x, B_w1, B_b1, B_w2):
    def _A_ref(x, c_kv, w_q, w_uk, w_uv, w_o):
        B, Sq, M = x.shape[0], x.shape[1], x.shape[2]
        Sk = c_kv.shape[1]
        H, D = w_q.shape[1], w_q.shape[2]
        q = jnp.einsum("bqm,mhd->bhqd", x, w_q)
        k = jnp.einsum("bkc,chd->bhkd", c_kv, w_uk)
        v = jnp.einsum("bkc,chd->bhkd", c_kv, w_uv)
        scores = jnp.einsum("bhqd,bhkd->bhqk", q, k) * (D ** -0.5)
        off = Sk - Sq
        qi = jnp.arange(Sq)[:, None]
        kj = jnp.arange(Sk)[None, :]
        cmask = kj <= (qi + off)
        scores = jnp.where(cmask[None, None], scores, -1e9)
        p = _softmax(scores, axis=-1)
        ctx = jnp.einsum("bhqk,bhkd->bhqd", p, v)
        return jnp.einsum("bhqd,hdm->bqm", ctx, w_o)

    def _B_ref(x, w1, b1, w2):
        h = jnp.einsum("bsd,df->bsf", x, w1) + b1
        sp = jnp.log1p(jnp.exp(-jnp.abs(h))) + jnp.where(h > 0, h, jnp.zeros_like(h))
        act = h * jnp.tanh(sp)
        return jnp.einsum("bsf,fd->bsd", act, w2)

    x = A_x
    h = x + _A_ref(_layernorm(x, axis=-1), A_c_kv, A_w_q, A_w_uk, A_w_uv, A_w_o)
    h2 = h + _B_ref(_layernorm(h, axis=-1), B_w1, B_b1, B_w2)
    return h2
```

```python
import functools
import numpy as np
import jax
import jax.numpy as jnp
from jax import lax
import jax.experimental.pallas as pl
import jax.experimental.pallas.tpu as pltpu

B, H, SK, D, M, DC, F = 2, 32, 8192, 128, 512, 512, 1792
EPS = 1e-5
LOG2E = 1.4426950408889634
NEG_BIG = -1e30

f32 = jnp.float32
bf16 = jnp.bfloat16
u32 = jnp.uint32

CW = 128
NW = M // CW
CK = 1024
NK = SK // CK
CO = 8
NO = H // CO
C1 = 128
N1 = M // C1
C2 = 256
N2 = F // C2

NN = (((1,), (1,)), ((), ()))


def _layernorm8(x8):
    m = jnp.mean(x8, axis=-1, keepdims=True)
    c = x8 - m
    v = jnp.mean(c * c, axis=-1, keepdims=True)
    return c / jnp.sqrt(v + EPS)


def _pack(a):
    return pltpu.bitcast(a.astype(bf16), u32)


def _kernel(x_hbm, ckv_hbm, wq_hbm, wuk_hbm, wuv_hbm, wo_hbm, w1_hbm, b1_hbm, w2_hbm, o_ref,
            xb, ckv, wq, wuk, wuv, wo, w1, b1b, w2, e_ref, xp_ref, qa_ref, cc_ref, cw_ref, sems):
    S_X, S_Q = 0, 1
    S_UK = S_Q + NW
    S_KV = S_UK + NW
    S_UV = S_KV + B * NK
    S_O = S_UV + NW
    S_1 = S_O + NO
    S_B1 = S_1 + N1
    S_2 = S_B1 + 1

    def rows(src, dst, size, base):
        def mk(i):
            off = i * size if isinstance(i, int) else pl.multiple_of(i * size, size)
            return pltpu.make_async_copy(src.at[pl.ds(off, size)], dst.at[pl.ds(off, size)], sems.at[base + i])
        return mk

    cp_x = pltpu.make_async_copy(x_hbm, xb, sems.at[S_X])
    cp_q = rows(wq_hbm, wq, CW, S_Q)
    cp_uk = rows(wuk_hbm, wuk, CW, S_UK)
    cp_uv = rows(wuv_hbm, wuv, CW, S_UV)
    cp_o = rows(wo_hbm, wo, CO, S_O)
    cp_1 = rows(w1_hbm, w1, C1, S_1)
    cp_2 = rows(w2_hbm, w2, C2, S_2)
    cp_b1 = pltpu.make_async_copy(b1_hbm, b1b, sems.at[S_B1])

    def cp_kv(b, i):
        off = i * CK if isinstance(i, int) else pl.multiple_of(i * CK, CK)
        return pltpu.make_async_copy(ckv_hbm.at[b, pl.ds(off, CK)], ckv.at[b, pl.ds(off, CK)], sems.at[S_KV + b * NK + i])

    cp_x.start()
    for i in range(NW):
        cp_q(i).start()
    for i in range(NW):
        cp_uk(i).start()
    for b in range(B):
        for i in range(NK):
            cp_kv(b, i).start()
    for i in range(NW):
        cp_uv(i).start()
    for i in range(NO):
        cp_o(i).start()
    for i in range(N1):
        cp_1(i).start()
    cp_b1.start()
    for i in range(N2):
        cp_2(i).start()

    L = CW * H

    for g in range(L // 512):
        lane = lax.broadcasted_iota(jnp.int32, (CW // 2, 512), 1) + g * 512
        row = lax.broadcasted_iota(jnp.int32, (CW // 2, 512), 0)
        c = lane >> 5
        one = jnp.where((c & 1) == 1, jnp.uint32(0x3F800000), jnp.uint32(0x3F80))
        e_ref[:, g * 512:(g + 1) * 512] = jnp.where((c >> 1) == row, one, jnp.uint32(0))

    def head_mask(width):
        lane = lax.broadcasted_iota(jnp.int32, (H, 128), 1)
        row = lax.broadcasted_iota(jnp.int32, (H, 128), 0)
        m = (lane & 31) == row
        return jnp.concatenate([m] * (width // 128), axis=1) if width > 128 else m

    def keep_diag(words):
        return jnp.where(head_mask(words.shape[1]), words, jnp.uint32(0))

    cp_x.wait()
    x2 = xb[...].astype(f32)
    par = lax.broadcasted_iota(jnp.int32, (8, M), 0) & 1
    x8 = jnp.where(par == 0, jnp.broadcast_to(x2[0:1], (8, M)), jnp.broadcast_to(x2[1:2], (8, M)))
    xn8 = _layernorm8(x8)
    lhs = jnp.concatenate([xn8[:, j * CW:(j + 1) * CW] for j in range(NW) for _ in range(2)], axis=0)
    lhs = lhs.astype(bf16)
    for g in range(L // 512):
        e = pltpu.bitcast(e_ref[:, g * 512:(g + 1) * 512], bf16)
        r = jnp.dot(lhs, e, preferred_element_type=f32)
        xp_ref[:, g * 512:(g + 1) * 512] = _pack(r)

    def q_body(j, acc):
        cp_q(j).wait()
        r0 = pl.multiple_of(j * 8, 8)
        m0 = pl.multiple_of(j * CW, CW)
        xpj = xp_ref[pl.ds(r0, 8), :]
        xw = keep_diag(jnp.concatenate([xpj] * 4, axis=0))
        w = wq[pl.ds(m0, CW)].reshape(L, D)
        return acc + jnp.dot(pltpu.bitcast(xw, bf16), w, preferred_element_type=f32)

    q = lax.fori_loop(0, NW, q_body, jnp.zeros((2 * H, D), f32))
    qb = (q * (D ** -0.5 * LOG2E)).astype(bf16)

    def qa_body(j, _):
        cp_uk(j).wait()
        m0 = pl.multiple_of(j * CW, CW)
        w = wuk[pl.ds(m0, CW)].reshape(L, D)
        r = lax.dot_general(qb, w, NN, preferred_element_type=f32)
        rm = pltpu.bitcast(keep_diag(_pack(r)), bf16)
        e = pltpu.bitcast(e_ref[...], bf16)
        qa = lax.dot_general(rm, e, NN, preferred_element_type=f32)
        wd = _pack(qa)
        lo = pltpu.bitcast(wd << 16, f32)
        hi = pltpu.bitcast(wd & jnp.uint32(0xFFFF0000), f32)
        qa_ref[0, j] = lo.astype(bf16)
        qa_ref[1, j] = hi.astype(bf16)
        return 0

    lax.fori_loop(0, NW, qa_body, 0)

    for b in range(B):
        qh = jnp.concatenate([qa_ref[b, j] for j in range(NW)], axis=1)

        def kv_body(i, carry, b=b, qh=qh):
            m_old, l_old, acc = carry
            cp_kv(b, i).wait()
            k0 = pl.multiple_of(i * CK, CK)
            c = ckv[b, pl.ds(k0, CK), :]
            s = lax.dot_general(qh, c, NN, preferred_element_type=f32)
            m_new = jnp.maximum(m_old, jnp.max(s, axis=1, keepdims=True))
            alpha = jnp.exp2(m_old - m_new)
            p = jnp.exp2(s - m_new)
            ps = p[:, 0:128]
            for t in range(1, CK // 128):
                ps = ps + p[:, t * 128:(t + 1) * 128]
            l_new = alpha * l_old + ps
            acc = alpha * acc + jnp.dot(p.astype(bf16), c, preferred_element_type=f32)
            return m_new, l_new, acc

        m, l, acc = lax.fori_loop(
            0, NK, kv_body,
            (jnp.full((H, 1), NEG_BIG, f32), jnp.zeros((H, 128), f32), jnp.zeros((H, DC), f32)))
        cc_ref[b] = acc / jnp.sum(l, axis=1, keepdims=True)

    c0 = pltpu.bitcast(cc_ref[0].astype(bf16).astype(f32), u32)
    c1 = pltpu.bitcast(cc_ref[1].astype(bf16).astype(f32), u32)
    cw_ref[...] = (c1 & jnp.uint32(0xFFFF0000)) | (c0 >> 16)

    def ctx_step(j, acc):
        lhs_c = pltpu.bitcast(cw_ref[:, j * CW:(j + 1) * CW], bf16)
        e = pltpu.bitcast(e_ref[...], bf16)
        y = jnp.dot(lhs_c, e, preferred_element_type=f32)
        ym = pltpu.bitcast(keep_diag(_pack(y)), bf16)
        cp_uv(j).wait()
        w = wuv[pl.ds(j * CW, CW)].reshape(L, D)
        return acc + jnp.dot(ym, w, preferred_element_type=f32)

    ctx = jnp.zeros((2 * H, D), f32)
    for j in range(NW):
        ctx = ctx_step(j, ctx)
    ctxw = _pack(ctx)

    sub8 = lax.broadcasted_iota(jnp.int32, (8, D), 0)
    acc_o = jnp.zeros((16, M), f32)
    for i in range(NO):
        cp_o(i).wait()
        grp = ctxw[8 * i:8 * (i + 1)]
        lhs_o = jnp.concatenate(
            [jnp.where(sub8 == s, grp, jnp.uint32(0)) for s in range(CO)], axis=1)
        w = wo[pl.ds(i * CO, CO)].reshape(CO * D, M)
        acc_o = acc_o + jnp.dot(pltpu.bitcast(lhs_o, bf16), w, preferred_element_type=f32)
    a8 = acc_o[0:8] + acc_o[8:16]
    a8 = a8 + pltpu.roll(a8, 4, 0)
    a8 = a8 + pltpu.roll(a8, 2, 0)
    h8 = x8 + a8

    hn8 = _layernorm8(h8)
    hb = jnp.concatenate([hn8, hn8], axis=0).astype(bf16)
    acc1 = jnp.zeros((16, F), f32)
    for i in range(N1):
        cp_1(i).wait()
        acc1 = acc1 + jnp.dot(hb[:, i * C1:(i + 1) * C1], w1[pl.ds(i * C1, C1), :], preferred_element_type=f32)
    cp_b1.wait()
    z = acc1[0:8] + b1b[...].astype(f32).reshape(1, F)
    sp = jnp.log1p(jnp.exp(-jnp.abs(z))) + jnp.where(z > 0, z, 0.0)
    act = z * jnp.tanh(sp)
    ab = jnp.concatenate([act, act], axis=0).astype(bf16)
    acc2 = jnp.zeros((16, M), f32)
    for i in range(N2):
        cp_2(i).wait()
        acc2 = acc2 + jnp.dot(ab[:, i * C2:(i + 1) * C2], w2[pl.ds(i * C2, C2), :], preferred_element_type=f32)
    out8 = h8 + acc2[0:8]
    o_ref[...] = out8[0:2].astype(o_ref.dtype)


@jax.jit
def pallas_sequential_preLN__compressed_kv_cla__dense_activation_mish__decode_kernel(A_x, A_c_kv, A_w_q, A_w_uk, A_w_uv, A_w_o, B_x, B_w1, B_b1, B_w2):
    del B_x
    hbm = pl.BlockSpec(memory_space=pltpu.HBM)
    nsem = 1 + 3 * NW + B * NK + NO + N1 + 1 + N2
    out = pl.pallas_call(
        _kernel,
        out_shape=jax.ShapeDtypeStruct((B, M), A_x.dtype),
        in_specs=[hbm] * 9,
        out_specs=pl.BlockSpec(memory_space=pltpu.VMEM),
        scratch_shapes=[
            pltpu.VMEM((B, M), bf16),
            pltpu.VMEM((B, SK, DC), bf16),
            pltpu.VMEM((M, H, D), bf16),
            pltpu.VMEM((DC, H, D), bf16),
            pltpu.VMEM((DC, H, D), bf16),
            pltpu.VMEM((H, D, M), bf16),
            pltpu.VMEM((M, F), bf16),
            pltpu.VMEM((F,), bf16),
            pltpu.VMEM((F, M), bf16),
            pltpu.VMEM((CW // 2, CW * H), u32),
            pltpu.VMEM((NW * 8, CW * H), u32),
            pltpu.VMEM((B, NW, H, CW), bf16),
            pltpu.VMEM((B, H, DC), f32),
            pltpu.VMEM((H, DC), u32),
            pltpu.SemaphoreType.DMA((nsem,)),
        ],
        compiler_params=pltpu.CompilerParams(vmem_limit_bytes=64 * 1024 * 1024),
    )(A_x.reshape(B, M), A_c_kv, A_w_q, A_w_uk, A_w_uv, A_w_o, B_w1, B_b1, B_w2)
    return out.reshape(A_x.shape)
```

```python
import functools

import jax
import jax.numpy as jnp
import numpy as np
from jax import lax
import jax.experimental.pallas as pl
import jax.experimental.pallas.tpu as pltpu

EPS = 1e-5
LOG2E = 1.4426950408889634
NEG_BIG = -1e30

f32 = jnp.float32
bf16 = jnp.bfloat16
u32 = jnp.uint32

HI16 = np.uint32(0xFFFF0000)
ONE_LO = np.uint32(0x00003F80)
ONE_HI = np.uint32(0x3F800000)
ZERO_U32 = np.uint32(0)

CW = 128
CK = 1024
CO = 8
C1 = 128

NT = (((1,), (1,)), ((), ()))


def _w2_chunks(f):
    sizes = [256] * ((f - 256) // 256)
    sizes += [128] * ((f - sum(sizes)) // 128)
    offs = np.cumsum([0] + sizes)
    return [(int(o), int(s)) for o, s in zip(offs, sizes)]


def _layernorm(x):
    mean = jnp.mean(x, axis=-1, keepdims=True)
    cen = x - mean
    var = jnp.mean(cen * cen, axis=-1, keepdims=True)
    return cen / jnp.sqrt(var + EPS)


def _pack(a):
    return pltpu.bitcast(a.astype(bf16), u32)


def _body(x_hbm, ckv_hbm, wq_hbm, wuk_hbm, wuv_hbm, wo_hbm, w1_hbm, b1_hbm, w2_hbm,
          xb, ckv, wq, wuk, wuv, wo, w1, b1, w2, e_ref, xp_ref, qa_ref, cc_ref, ob, cp_out, sems):
    B, SK, DC = ckv.shape
    M, H, D = wq.shape
    F = w1.shape[1]
    NQ, NC, NK, NO, N1 = M // CW, DC // CW, SK // CK, H // CO, M // C1
    L = CW * H
    w2_chunks = _w2_chunks(F)

    sem = iter(range(sems.shape[0]))

    def chunked(src, dst, n, size):
        base = [next(sem) for _ in range(n)][0]

        def mk(i):
            off = i * size if isinstance(i, int) else pl.multiple_of(i * size, size)
            return pltpu.make_async_copy(
                src.at[pl.ds(off, size)], dst.at[pl.ds(off, size)], sems.at[base + i])
        return mk

    cp_x = pltpu.make_async_copy(x_hbm, xb, sems.at[next(sem)])
    cp_q = chunked(wq_hbm, wq, NQ, CW)
    cp_uk = chunked(wuk_hbm, wuk, NC, CW)
    cp_kv = [chunked(ckv_hbm.at[b], ckv.at[b], NK, CK) for b in range(B)]
    cp_uv = chunked(wuv_hbm, wuv, NC, CW)
    cp_o = chunked(wo_hbm, wo, NO, CO)
    cp_1 = chunked(w1_hbm, w1, N1, C1)
    cp_b1 = pltpu.make_async_copy(b1_hbm, b1, sems.at[next(sem)])
    cp_2 = [pltpu.make_async_copy(w2_hbm.at[pl.ds(o, s)], w2.at[pl.ds(o, s)], sems.at[next(sem)])
            for o, s in w2_chunks]

    cp_x.start()
    for mk, n in [(cp_q, NQ), (cp_uk, NC)] + [(c, NK) for c in cp_kv] + [(cp_uv, NC), (cp_o, NO), (cp_1, N1)]:
        for i in range(n):
            mk(i).start()
    cp_b1.start()
    for c in cp_2:
        c.start()

    for g in range(L // 512):
        lane = lax.broadcasted_iota(jnp.int32, (CW // 2, 512), 1) + g * 512
        word = lax.broadcasted_iota(jnp.int32, (CW // 2, 512), 0)
        col = lane >> 5
        one = jnp.where((col & 1) == 1, ONE_HI, ONE_LO)
        e_ref[:, g * 512:(g + 1) * 512] = jnp.where((col >> 1) == word, one, ZERO_U32)

    def keep_diag(words):
        lane = lax.broadcasted_iota(jnp.int32, (H, 128), 1)
        row = lax.broadcasted_iota(jnp.int32, (H, 128), 0)
        diag = jnp.concatenate([(lane & (H - 1)) == row] * (words.shape[1] // 128), axis=1)
        return jnp.where(diag, words, ZERO_U32)

    cp_x.wait()
    x2 = xb[...].astype(f32)
    odd = (lax.broadcasted_iota(jnp.int32, (8, M), 0) & 1) == 1
    x8 = jnp.where(odd, jnp.broadcast_to(x2[1:2], (8, M)), jnp.broadcast_to(x2[0:1], (8, M)))
    xn8 = _layernorm(x8)
    xn = jnp.concatenate([xn8[:, j * CW:(j + 1) * CW] for j in range(NQ) for _ in range(2)], axis=0)
    xn = xn.astype(bf16)
    for g in range(L // 512):
        e = pltpu.bitcast(e_ref[:, g * 512:(g + 1) * 512], bf16)
        xp_ref[:, g * 512:(g + 1) * 512] = _pack(jnp.dot(xn, e, preferred_element_type=f32))

    def q_step(j, acc):
        cp_q(j).wait()
        xpj = xp_ref[pl.ds(pl.multiple_of(j * 8, 8), 8), :]
        lhs = keep_diag(jnp.concatenate([xpj] * (H // 8), axis=0))
        w = wq[pl.ds(pl.multiple_of(j * CW, CW), CW)].reshape(L, D)
        return acc + jnp.dot(pltpu.bitcast(lhs, bf16), w, preferred_element_type=f32)

    q = lax.fori_loop(0, NQ, q_step, jnp.zeros((B * H, D), f32))
    qb = (q * (D ** -0.5 * LOG2E)).astype(bf16)

    def qa_step(j, carry):
        cp_uk(j).wait()
        w = wuk[pl.ds(pl.multiple_of(j * CW, CW), CW)].reshape(L, D)
        r = lax.dot_general(qb, w, NT, preferred_element_type=f32)
        r = pltpu.bitcast(keep_diag(_pack(r)), bf16)
        e = pltpu.bitcast(e_ref[...], bf16)
        words = _pack(lax.dot_general(r, e, NT, preferred_element_type=f32))
        qa_ref[0, j] = pltpu.bitcast(words << 16, f32).astype(bf16)
        qa_ref[1, j] = pltpu.bitcast(words & HI16, f32).astype(bf16)
        return carry

    lax.fori_loop(0, NC, qa_step, 0)

    for b in range(B):
        qh = jnp.concatenate([qa_ref[b, j] for j in range(NC)], axis=1)

        def kv_step(i, carry, b=b, qh=qh):
            m_old, l_old, acc = carry
            cp_kv[b](i).wait()
            c = ckv[b, pl.ds(pl.multiple_of(i * CK, CK), CK), :]
            s = lax.dot_general(qh, c, NT, preferred_element_type=f32)
            m_new = jnp.maximum(m_old, jnp.max(s, axis=1, keepdims=True))
            alpha = jnp.exp2(m_old - m_new)
            p = jnp.exp2(s - m_new)
            l_blk = functools.reduce(jnp.add, [p[:, t:t + 128] for t in range(0, CK, 128)])
            acc = alpha * acc + jnp.dot(p.astype(bf16), c, preferred_element_type=f32)
            return m_new, alpha * l_old + l_blk, acc

        init = (jnp.full((H, 1), NEG_BIG, f32), jnp.zeros((H, 128), f32), jnp.zeros((H, DC), f32))
        _, l, acc = lax.fori_loop(0, NK, kv_step, init)
        cc_ref[b] = acc / jnp.sum(l, axis=1, keepdims=True)

    cc = [pltpu.bitcast(cc_ref[b].astype(bf16).astype(f32), u32) for b in range(B)]
    cc = pltpu.bitcast((cc[1] & HI16) | (cc[0] >> 16), bf16)
    ctx = jnp.zeros((B * H, D), f32)
    for j in range(NC):
        e = pltpu.bitcast(e_ref[...], bf16)
        y = jnp.dot(cc[:, j * CW:(j + 1) * CW], e, preferred_element_type=f32)
        y = pltpu.bitcast(keep_diag(_pack(y)), bf16)
        cp_uv(j).wait()
        w = wuv[j * CW:(j + 1) * CW].reshape(L, D)
        ctx = ctx + jnp.dot(y, w, preferred_element_type=f32)
    ctx = _pack(ctx)

    sub = lax.broadcasted_iota(jnp.int32, (CO, D), 0)
    proj = jnp.zeros((16, M), f32)
    for i in range(NO):
        cp_o(i).wait()
        grp = ctx[i * CO:(i + 1) * CO]
        lhs = jnp.concatenate([jnp.where(sub == s, grp, ZERO_U32) for s in range(CO)], axis=1)
        w = wo[i * CO:(i + 1) * CO].reshape(CO * D, M)
        proj = proj + jnp.dot(pltpu.bitcast(lhs, bf16), w, preferred_element_type=f32)
    proj = proj[0:8] + proj[8:16]
    proj = proj + pltpu.roll(proj, 4, 0)
    proj = proj + pltpu.roll(proj, 2, 0)
    h8 = x8 + proj

    hn = _layernorm(h8)
    hn = jnp.concatenate([hn, hn], axis=0).astype(bf16)
    z = jnp.zeros((16, F), f32)
    for i in range(N1):
        cp_1(i).wait()
        z = z + jnp.dot(hn[:, i * C1:(i + 1) * C1], w1[i * C1:(i + 1) * C1, :], preferred_element_type=f32)
    cp_b1.wait()
    z = z[0:8] + b1[...].astype(f32).reshape(1, F)
    softplus = jnp.log1p(jnp.exp(-jnp.abs(z))) + jnp.where(z > 0, z, 0.0)
    act = z * jnp.tanh(softplus)
    act = jnp.concatenate([act, act], axis=0).astype(bf16)
    out = h8
    for cp, (o, s) in zip(cp_2, w2_chunks):
        cp.wait()
        out = out + jnp.dot(act[:, o:o + s], w2[o:o + s, :], preferred_element_type=f32)[0:8]
    ob[...] = out[0:B].astype(ob.dtype)
    cp_out.start()


def _kernel(*refs):
    ins, o_hbm, scratch, ob, osem = refs[:9], refs[9], refs[10:-2], refs[-2], refs[-1]
    _, ckv, wq, _, _, _, w1, _, _ = scratch[:9]
    nsem = (2 + wq.shape[0] // CW + 2 * (ckv.shape[2] // CW) + ckv.shape[0] * (ckv.shape[1] // CK)
            + wq.shape[1] // CO + wq.shape[0] // C1 + len(_w2_chunks(w1.shape[1])))
    cp_out = pltpu.make_async_copy(ob, o_hbm, osem)
    pl.run_scoped(lambda sems: _body(*ins, *scratch, ob, cp_out, sems), pltpu.SemaphoreType.DMA((nsem,)))
    cp_out.wait()


@jax.jit
def pallas_sequential_preLN__compressed_kv_cla__dense_activation_mish__decode_kernel(
    A_x: jax.Array,
    A_c_kv: jax.Array,
    A_w_q: jax.Array,
    A_w_uk: jax.Array,
    A_w_uv: jax.Array,
    A_w_o: jax.Array,
    B_x: jax.Array,
    B_w1: jax.Array,
    B_b1: jax.Array,
    B_w2: jax.Array,
):
    del B_x
    B, Sq, M = A_x.shape
    _, H, D = A_w_q.shape
    DC = A_c_kv.shape[2]
    assert (B, Sq, H, D) == (2, 1, 32, 128), "the row packing assumes 2 batch entries, 1 query and 32 heads of 128"
    ins = (A_x.reshape(B, M), A_c_kv, A_w_q, A_w_uk, A_w_uv, A_w_o, B_w1, B_b1, B_w2)
    hbm = pl.BlockSpec(memory_space=pltpu.HBM)
    out = pl.pallas_call(
        _kernel,
        out_shape=jax.ShapeDtypeStruct((B, M), A_x.dtype),
        in_specs=[hbm] * len(ins),
        out_specs=hbm,
        scratch_shapes=[pltpu.VMEM(a.shape, a.dtype) for a in ins] + [
            pltpu.VMEM((CW // 2, CW * H), u32),
            pltpu.VMEM((M // CW * 8, CW * H), u32),
            pltpu.VMEM((B, DC // CW, H, CW), bf16),
            pltpu.VMEM((B, H, DC), f32),
            pltpu.VMEM((B, M), A_x.dtype),
            pltpu.SemaphoreType.DMA(()),
        ],
        compiler_params=pltpu.CompilerParams(vmem_limit_bytes=64 * 1024 * 1024),
    )(*ins)
    return out.reshape(A_x.shape)
```

```python
import functools

import jax
import jax.numpy as jnp
import numpy as np
from jax import lax
import jax.experimental.pallas as pl
import jax.experimental.pallas.tpu as pltpu

EPS = 1e-5
LOG2E = 1.4426950408889634
NEG_BIG = -1e30

f32 = jnp.float32
bf16 = jnp.bfloat16
u32 = jnp.uint32

HI16 = np.uint32(0xFFFF0000)
ONE_LO = np.uint32(0x00003F80)
ONE_HI = np.uint32(0x3F800000)
ZERO_U32 = np.uint32(0)

CW = 128
CK = 1024
CO = 8
C1 = 128
SIDE = 896
TAIL = 128

NT = (((1,), (1,)), ((), ()))


def _w2_chunks(f):
    sizes = [256] * ((f - SIDE - TAIL - 256) // 256)
    sizes += [128] * ((f - SIDE - TAIL - sum(sizes)) // 128)
    sizes += [TAIL // 2] * 2
    offs = SIDE + np.cumsum([0] + sizes)
    return [(int(o), int(s)) for o, s in zip(offs, sizes)]


def _layernorm(x):
    mean = jnp.mean(x, axis=-1, keepdims=True)
    cen = x - mean
    var = jnp.mean(cen * cen, axis=-1, keepdims=True)
    return cen / jnp.sqrt(var + EPS)


def _pack(a):
    return pltpu.bitcast(a.astype(bf16), u32)


def _body(x_hbm, ckv_hbm, wq_hbm, wuk_hbm, wuv_hbm, wo_hbm, w1_hbm, b1_hbm, w2_hbm,
          xb, ckv, wq, wuk, wuv, wo, w1, b1, w2, e_ref, xp_ref, qa_ref, cc_ref, side_smem, side_vmem, at_ref,
          ob, cp_out, sems):
    B, SK, DC = ckv.shape
    M, H, D = wq.shape
    F = w1.shape[1]
    NQ, NC, NK, NO, N1 = M // CW, DC // CW, SK // CK, H // CO, M // C1
    L = CW * H
    w2_chunks = _w2_chunks(F)

    sem = iter(range(sems.shape[0]))

    def chunked(src, dst, n, size):
        base = [next(sem) for _ in range(n)][0]

        def mk(i):
            off = i * size if isinstance(i, int) else pl.multiple_of(i * size, size)
            return pltpu.make_async_copy(
                src.at[pl.ds(off, size)], dst.at[pl.ds(off, size)], sems.at[base + i])
        return mk

    cp_x = pltpu.make_async_copy(x_hbm, xb, sems.at[next(sem)])
    cp_q = chunked(wq_hbm, wq, NQ, CW)
    cp_uk = chunked(wuk_hbm, wuk, NC, CW)
    cp_kv = [chunked(ckv_hbm.at[b], ckv.at[b], NK, CK) for b in range(B)]
    cp_uv = chunked(wuv_hbm, wuv, NC, CW)
    cp_o = chunked(wo_hbm, wo, NO, CO)
    cp_1 = chunked(w1_hbm, w1, N1, C1)
    cp_b1 = pltpu.make_async_copy(b1_hbm, b1, sems.at[next(sem)])
    cp_2 = [pltpu.make_async_copy(w2_hbm.at[pl.ds(o, s)], w2.at[pl.ds(o, s)], sems.at[next(sem)])
            for o, s in w2_chunks]
    side_in = pltpu.make_async_copy(w2_hbm.bitcast(u32).at[pl.ds(0, SIDE // 2)], side_smem, sems.at[next(sem)])
    side_out = pltpu.make_async_copy(side_smem, side_vmem, sems.at[next(sem)])

    side_in.start()
    cp_x.start()
    for mk, n in [(cp_q, NQ), (cp_uk, NC)] + [(c, NK) for c in cp_kv] + [(cp_uv, NC), (cp_o, NO), (cp_1, N1)]:
        for i in range(n):
            mk(i).start()
    cp_b1.start()
    for c in cp_2:
        c.start()

    for g in range(L // 512):
        lane = lax.broadcasted_iota(jnp.int32, (CW // 2, 512), 1) + g * 512
        word = lax.broadcasted_iota(jnp.int32, (CW // 2, 512), 0)
        col = lane >> 5
        one = jnp.where((col & 1) == 1, ONE_HI, ONE_LO)
        e_ref[:, g * 512:(g + 1) * 512] = jnp.where((col >> 1) == word, one, ZERO_U32)

    def keep_diag(words):
        lane = lax.broadcasted_iota(jnp.int32, (H, 128), 1)
        row = lax.broadcasted_iota(jnp.int32, (H, 128), 0)
        diag = jnp.concatenate([(lane & (H - 1)) == row] * (words.shape[1] // 128), axis=1)
        return jnp.where(diag, words, ZERO_U32)

    cp_x.wait()
    x2 = xb[...].astype(f32)
    odd = (lax.broadcasted_iota(jnp.int32, (8, M), 0) & 1) == 1
    x8 = jnp.where(odd, jnp.broadcast_to(x2[1:2], (8, M)), jnp.broadcast_to(x2[0:1], (8, M)))
    xn8 = _layernorm(x8)
    xn = jnp.concatenate([xn8[:, j * CW:(j + 1) * CW] for j in range(NQ) for _ in range(2)], axis=0)
    xn = xn.astype(bf16)
    for g in range(L // 512):
        e = pltpu.bitcast(e_ref[:, g * 512:(g + 1) * 512], bf16)
        xp_ref[:, g * 512:(g + 1) * 512] = _pack(jnp.dot(xn, e, preferred_element_type=f32))

    def q_step(j, acc):
        cp_q(j).wait()
        xpj = xp_ref[pl.ds(pl.multiple_of(j * 8, 8), 8), :]
        lhs = keep_diag(jnp.concatenate([xpj] * (H // 8), axis=0))
        w = wq[pl.ds(pl.multiple_of(j * CW, CW), CW)].reshape(L, D)
        return acc + jnp.dot(pltpu.bitcast(lhs, bf16), w, preferred_element_type=f32)

    q = lax.fori_loop(0, NQ, q_step, jnp.zeros((B * H, D), f32))
    qb = (q * (D ** -0.5 * LOG2E)).astype(bf16)

    def qa_step(j, carry):
        cp_uk(j).wait()
        w = wuk[pl.ds(pl.multiple_of(j * CW, CW), CW)].reshape(L, D)
        r = lax.dot_general(qb, w, NT, preferred_element_type=f32)
        r = pltpu.bitcast(keep_diag(_pack(r)), bf16)
        e = pltpu.bitcast(e_ref[...], bf16)
        words = _pack(lax.dot_general(r, e, NT, preferred_element_type=f32))
        qa_ref[0, j] = pltpu.bitcast(words << 16, f32).astype(bf16)
        qa_ref[1, j] = pltpu.bitcast(words & HI16, f32).astype(bf16)
        return carry

    lax.fori_loop(0, NC, qa_step, 0)

    for b in range(B):
        if b == B - 1:
            side_in.wait()
            side_out.start()
        qh = jnp.concatenate([qa_ref[b, j] for j in range(NC)], axis=1)

        def kv_step(i, carry, b=b, qh=qh):
            m_old, l_old, acc = carry
            cp_kv[b](i).wait()
            c = ckv[b, pl.ds(pl.multiple_of(i * CK, CK), CK), :]
            s = lax.dot_general(qh, c, NT, preferred_element_type=f32)
            m_new = jnp.maximum(m_old, jnp.max(s, axis=1, keepdims=True))
            alpha = jnp.exp2(m_old - m_new)
            p = jnp.exp2(s - m_new)
            l_blk = functools.reduce(jnp.add, [p[:, t:t + 128] for t in range(0, CK, 128)])
            acc = alpha * acc + jnp.dot(p.astype(bf16), c, preferred_element_type=f32)
            return m_new, alpha * l_old + l_blk, acc

        init = (jnp.full((H, 1), NEG_BIG, f32), jnp.zeros((H, 128), f32), jnp.zeros((H, DC), f32))
        _, l, acc = lax.fori_loop(0, NK, kv_step, init)
        cc_ref[b] = acc / jnp.sum(l, axis=1, keepdims=True)

    cc = [pltpu.bitcast(cc_ref[b].astype(bf16).astype(f32), u32) for b in range(B)]
    cc = pltpu.bitcast((cc[1] & HI16) | (cc[0] >> 16), bf16)
    ctx = jnp.zeros((B * H, D), f32)
    for j in range(NC):
        e = pltpu.bitcast(e_ref[...], bf16)
        y = jnp.dot(cc[:, j * CW:(j + 1) * CW], e, preferred_element_type=f32)
        y = pltpu.bitcast(keep_diag(_pack(y)), bf16)
        cp_uv(j).wait()
        w = wuv[j * CW:(j + 1) * CW].reshape(L, D)
        ctx = ctx + jnp.dot(y, w, preferred_element_type=f32)
    ctx = _pack(ctx)

    sub = lax.broadcasted_iota(jnp.int32, (CO, D), 0)
    proj = jnp.zeros((16, M), f32)
    for i in range(NO):
        cp_o(i).wait()
        grp = ctx[i * CO:(i + 1) * CO]
        lhs = jnp.concatenate([jnp.where(sub == s, grp, ZERO_U32) for s in range(CO)], axis=1)
        w = wo[i * CO:(i + 1) * CO].reshape(CO * D, M)
        proj = proj + jnp.dot(pltpu.bitcast(lhs, bf16), w, preferred_element_type=f32)
    proj = proj[0:8] + proj[8:16]
    proj = proj + pltpu.roll(proj, 4, 0)
    proj = proj + pltpu.roll(proj, 2, 0)
    h8 = x8 + proj

    hn = _layernorm(h8)
    hn = jnp.concatenate([hn, hn], axis=0).astype(bf16)
    z = jnp.zeros((16, F), f32)
    for i in range(N1):
        cp_1(i).wait()
        z = z + jnp.dot(hn[:, i * C1:(i + 1) * C1], w1[i * C1:(i + 1) * C1, :], preferred_element_type=f32)
    cp_b1.wait()
    z = z[0:8] + b1[...].astype(f32).reshape(1, F)
    softplus = jnp.log1p(jnp.exp(-jnp.abs(z))) + jnp.where(z > 0, z, 0.0)
    act = z * jnp.tanh(softplus)
    for b in range(B):
        at_ref[b] = jnp.broadcast_to(act[b:b + 1, F - TAIL:], (128, TAIL)).T
    act = jnp.concatenate([act, act], axis=0).astype(bf16)

    side_out.wait()
    w = pltpu.bitcast(side_vmem[...], bf16)
    out = h8 + jnp.dot(act[:, :SIDE], w, preferred_element_type=f32)[0:8]
    tail = [[None] * (M // 128) for _ in range(B)]
    for cp, (o, s) in zip(cp_2, w2_chunks):
        cp.wait()
        if o < F - TAIL:
            out = out + jnp.dot(act[:, o:o + s], w2[o:o + s, :], preferred_element_type=f32)[0:8]
            continue
        for r in range(o, o + s, 16):
            a = [at_ref[b, r - (F - TAIL):r - (F - TAIL) + 16, :] for b in range(B)]
            for t in range(M // 128):
                w = w2[r:r + 16, t * 128:(t + 1) * 128].astype(f32)
                for b in range(B):
                    prod = w * a[b]
                    prod = prod[0:8] + prod[8:16]
                    tail[b][t] = prod if tail[b][t] is None else tail[b][t] + prod
    tail = [jnp.concatenate(tail[b], axis=1) for b in range(B)]
    tail = jnp.where(odd, tail[1] + pltpu.roll(tail[1], 1, 0), tail[0] + pltpu.roll(tail[0], 7, 0))
    tail = tail + pltpu.roll(tail, 2, 0)
    tail = tail + pltpu.roll(tail, 4, 0)
    out = out + tail
    ob[...] = out[0:B].astype(ob.dtype)
    cp_out.start()


def _kernel(*refs):
    ins, o_hbm, scratch, ob, osem = refs[:9], refs[9], refs[10:-2], refs[-2], refs[-1]
    _, ckv, wq, _, _, _, w1, _, _ = scratch[:9]
    nsem = (4 + wq.shape[0] // CW + 2 * (ckv.shape[2] // CW) + ckv.shape[0] * (ckv.shape[1] // CK)
            + wq.shape[1] // CO + wq.shape[0] // C1 + len(_w2_chunks(w1.shape[1])))
    cp_out = pltpu.make_async_copy(ob, o_hbm, osem)
    pl.run_scoped(lambda sems: _body(*ins, *scratch, ob, cp_out, sems), pltpu.SemaphoreType.DMA((nsem,)))
    cp_out.wait()


@jax.jit
def pallas_sequential_preLN__compressed_kv_cla__dense_activation_mish__decode_kernel(
    A_x: jax.Array,
    A_c_kv: jax.Array,
    A_w_q: jax.Array,
    A_w_uk: jax.Array,
    A_w_uv: jax.Array,
    A_w_o: jax.Array,
    B_x: jax.Array,
    B_w1: jax.Array,
    B_b1: jax.Array,
    B_w2: jax.Array,
):
    del B_x
    B, Sq, M = A_x.shape
    _, H, D = A_w_q.shape
    DC = A_c_kv.shape[2]
    assert (B, Sq, H, D) == (2, 1, 32, 128), "the row packing assumes 2 batch entries, 1 query and 32 heads of 128"
    ins = (A_x.reshape(B, M), A_c_kv, A_w_q, A_w_uk, A_w_uv, A_w_o, B_w1, B_b1, B_w2)
    hbm = pl.BlockSpec(memory_space=pltpu.HBM)
    out = pl.pallas_call(
        _kernel,
        out_shape=jax.ShapeDtypeStruct((B, M), A_x.dtype),
        in_specs=[hbm] * len(ins),
        out_specs=hbm,
        scratch_shapes=[pltpu.VMEM(a.shape, a.dtype) for a in ins] + [
            pltpu.VMEM((CW // 2, CW * H), u32),
            pltpu.VMEM((M // CW * 8, CW * H), u32),
            pltpu.VMEM((B, DC // CW, H, CW), bf16),
            pltpu.VMEM((B, H, DC), f32),
            pltpu.SMEM((SIDE // 2, M), u32),
            pltpu.VMEM((SIDE // 2, M), u32),
            pltpu.VMEM((B, TAIL, 128), f32),
            pltpu.VMEM((B, M), A_x.dtype),
            pltpu.SemaphoreType.DMA(()),
        ],
        compiler_params=pltpu.CompilerParams(vmem_limit_bytes=64 * 1024 * 1024),
    )(*ins)
    return out.reshape(A_x.shape)
```

```python
import functools

import jax
import jax.numpy as jnp
import numpy as np
from jax import lax
import jax.experimental.pallas as pl
import jax.experimental.pallas.tpu as pltpu

EPS = 1e-5
LOG2E = 1.4426950408889634
NEG_BIG = -1e30

f32 = jnp.float32
bf16 = jnp.bfloat16
u32 = jnp.uint32

HI16 = np.uint32(0xFFFF0000)
ONE_LO = np.uint32(0x00003F80)
ONE_HI = np.uint32(0x3F800000)
ZERO_U32 = np.uint32(0)

CW = 128
CK = 1024
CO = 8
C1 = 128
SIDE = 896
TAIL = 128

NT = (((1,), (1,)), ((), ()))


def _w2_chunks(f):
    sizes = [f - SIDE - TAIL - 256, 256, TAIL // 2, TAIL // 2]
    offs = SIDE + np.cumsum([0] + sizes)
    return [(int(o), int(s)) for o, s in zip(offs, sizes)]


def _layernorm(x):
    mean = jnp.mean(x, axis=-1, keepdims=True)
    cen = x - mean
    var = jnp.mean(cen * cen, axis=-1, keepdims=True)
    return cen / jnp.sqrt(var + EPS)


def _pack(a):
    return pltpu.bitcast(a.astype(bf16), u32)


def _body(x_hbm, ckv_hbm, wq_hbm, wuk_hbm, wuv_hbm, wo_hbm, w1_hbm, b1_hbm, w2_hbm,
          xb, ckv, wq, wuk, wuv, wo, w1, b1, w2, e_ref, xp_ref, qa_ref, cc_ref, side, at_ref,
          ob, cp_out, sems):
    B, SK, DC = ckv.shape
    M, H, D = wq.shape
    F = w1.shape[1]
    NQ, NC, NK, NO, N1 = M // CW, DC // CW, SK // CK, H // CO, M // C1
    L = CW * H
    w2_chunks = _w2_chunks(F)

    sem = iter(range(sems.shape[0]))

    def chunked(src, dst, n, size):
        base = [next(sem) for _ in range(n)][0]

        def mk(i):
            off = i * size if isinstance(i, int) else pl.multiple_of(i * size, size)
            return pltpu.make_async_copy(
                src.at[pl.ds(off, size)], dst.at[pl.ds(off, size)], sems.at[base + i])
        return mk

    cp_x = pltpu.make_async_copy(x_hbm, xb, sems.at[next(sem)])
    cp_q = chunked(wq_hbm, wq, NQ, CW)
    cp_uk = chunked(wuk_hbm, wuk, NC, CW)
    cp_kv = [chunked(ckv_hbm.at[b], ckv.at[b], NK, CK) for b in range(B)]
    cp_uv = chunked(wuv_hbm, wuv, NC, CW)
    cp_o = chunked(wo_hbm, wo, NO, CO)
    cp_1 = chunked(w1_hbm, w1, N1, C1)
    cp_b1 = pltpu.make_async_copy(b1_hbm, b1, sems.at[next(sem)])
    cp_2 = [pltpu.make_async_copy(w2_hbm.at[pl.ds(o, s)], w2.at[pl.ds(o, s)], sems.at[next(sem)])
            for o, s in w2_chunks]
    side_in = pltpu.make_async_copy(w2_hbm.at[pl.ds(0, SIDE)], side, sems.at[next(sem)])
    side_out = pltpu.make_async_copy(side, w2.at[pl.ds(0, SIDE)], sems.at[next(sem)])

    side_in.start()
    cp_x.start()
    for mk, n in [(cp_q, NQ), (cp_uk, NC)] + [(c, NK) for c in cp_kv] + [(cp_uv, NC), (cp_o, NO), (cp_1, N1)]:
        for i in range(n):
            mk(i).start()
    cp_b1.start()
    for c in cp_2:
        c.start()

    for g in range(L // 512):
        lane = lax.broadcasted_iota(jnp.int32, (CW // 2, 512), 1) + g * 512
        word = lax.broadcasted_iota(jnp.int32, (CW // 2, 512), 0)
        col = lane >> 5
        one = jnp.where((col & 1) == 1, ONE_HI, ONE_LO)
        e_ref[:, g * 512:(g + 1) * 512] = jnp.where((col >> 1) == word, one, ZERO_U32)

    def keep_diag(words):
        lane = lax.broadcasted_iota(jnp.int32, (H, 128), 1)
        row = lax.broadcasted_iota(jnp.int32, (H, 128), 0)
        diag = jnp.concatenate([(lane & (H - 1)) == row] * (words.shape[1] // 128), axis=1)
        return jnp.where(diag, words, ZERO_U32)

    cp_x.wait()
    x2 = xb[...].astype(f32)
    odd = (lax.broadcasted_iota(jnp.int32, (8, M), 0) & 1) == 1
    x8 = jnp.where(odd, jnp.broadcast_to(x2[1:2], (8, M)), jnp.broadcast_to(x2[0:1], (8, M)))
    xn8 = _layernorm(x8)
    xn = jnp.concatenate([xn8[:, j * CW:(j + 1) * CW] for j in range(NQ) for _ in range(2)], axis=0)
    xn = xn.astype(bf16)
    for g in range(L // 512):
        e = pltpu.bitcast(e_ref[:, g * 512:(g + 1) * 512], bf16)
        xp_ref[:, g * 512:(g + 1) * 512] = _pack(jnp.dot(xn, e, preferred_element_type=f32))

    def q_step(j, acc):
        cp_q(j).wait()
        xpj = xp_ref[pl.ds(pl.multiple_of(j * 8, 8), 8), :]
        lhs = keep_diag(jnp.concatenate([xpj] * (H // 8), axis=0))
        w = wq[pl.ds(pl.multiple_of(j * CW, CW), CW)].reshape(L, D)
        return acc + jnp.dot(pltpu.bitcast(lhs, bf16), w, preferred_element_type=f32)

    q = lax.fori_loop(0, NQ, q_step, jnp.zeros((B * H, D), f32))
    qb = (q * (D ** -0.5 * LOG2E)).astype(bf16)

    def qa_step(j, carry):
        cp_uk(j).wait()
        w = wuk[pl.ds(pl.multiple_of(j * CW, CW), CW)].reshape(L, D)
        r = lax.dot_general(qb, w, NT, preferred_element_type=f32)
        r = pltpu.bitcast(keep_diag(_pack(r)), bf16)
        e = pltpu.bitcast(e_ref[...], bf16)
        words = _pack(lax.dot_general(r, e, NT, preferred_element_type=f32))
        qa_ref[0, j] = pltpu.bitcast(words << 16, f32).astype(bf16)
        qa_ref[1, j] = pltpu.bitcast(words & HI16, f32).astype(bf16)
        return carry

    lax.fori_loop(0, NC, qa_step, 0)

    for b in range(B):
        if b == B - 1:
            side_in.wait()
            side_out.start()
        qh = jnp.concatenate([qa_ref[b, j] for j in range(NC)], axis=1)

        def kv_step(i, carry, b=b, qh=qh):
            m_old, l_old, acc = carry
            cp_kv[b](i).wait()
            c = ckv[b, pl.ds(pl.multiple_of(i * CK, CK), CK), :]
            s = lax.dot_general(qh, c, NT, preferred_element_type=f32)
            m_new = jnp.maximum(m_old, jnp.max(s, axis=1, keepdims=True))
            alpha = jnp.exp2(m_old - m_new)
            p = jnp.exp2(s - m_new)
            l_blk = functools.reduce(jnp.add, [p[:, t:t + 128] for t in range(0, CK, 128)])
            acc = alpha * acc + jnp.dot(p.astype(bf16), c, preferred_element_type=f32)
            return m_new, alpha * l_old + l_blk, acc

        init = (jnp.full((H, 1), NEG_BIG, f32), jnp.zeros((H, 128), f32), jnp.zeros((H, DC), f32))
        _, l, acc = lax.fori_loop(0, NK, kv_step, init)
        cc_ref[b] = acc / jnp.sum(l, axis=1, keepdims=True)

    cc = [pltpu.bitcast(cc_ref[b].astype(bf16).astype(f32), u32) for b in range(B)]
    cc = pltpu.bitcast((cc[1] & HI16) | (cc[0] >> 16), bf16)
    ctx = jnp.zeros((B * H, D), f32)
    for j in range(NC):
        e = pltpu.bitcast(e_ref[...], bf16)
        y = jnp.dot(cc[:, j * CW:(j + 1) * CW], e, preferred_element_type=f32)
        y = pltpu.bitcast(keep_diag(_pack(y)), bf16)
        cp_uv(j).wait()
        w = wuv[j * CW:(j + 1) * CW].reshape(L, D)
        ctx = ctx + jnp.dot(y, w, preferred_element_type=f32)
    ctx = _pack(ctx)

    sub = lax.broadcasted_iota(jnp.int32, (CO, D), 0)
    proj = jnp.zeros((16, M), f32)
    for i in range(NO):
        cp_o(i).wait()
        grp = ctx[i * CO:(i + 1) * CO]
        lhs = jnp.concatenate([jnp.where(sub == s, grp, ZERO_U32) for s in range(CO)], axis=1)
        w = wo[i * CO:(i + 1) * CO].reshape(CO * D, M)
        proj = proj + jnp.dot(pltpu.bitcast(lhs, bf16), w, preferred_element_type=f32)
    proj = proj[0:8] + proj[8:16]
    proj = proj + pltpu.roll(proj, 4, 0)
    proj = proj + pltpu.roll(proj, 2, 0)
    h8 = x8 + proj

    hn = _layernorm(h8)
    hn = jnp.concatenate([hn, hn], axis=0).astype(bf16)
    z = jnp.zeros((16, F), f32)
    for i in range(N1):
        cp_1(i).wait()
        z = z + jnp.dot(hn[:, i * C1:(i + 1) * C1], w1[i * C1:(i + 1) * C1, :], preferred_element_type=f32)
    cp_b1.wait()
    z = z[0:8] + b1[...].astype(f32).reshape(1, F)
    softplus = jnp.log1p(jnp.exp(-jnp.abs(z))) + jnp.where(z > 0, z, 0.0)
    act = z * jnp.tanh(softplus)
    for b in range(B):
        at_ref[b] = jnp.broadcast_to(act[b:b + 1, F - TAIL:], (128, TAIL)).T
    act = jnp.concatenate([act, act], axis=0).astype(bf16)

    side_out.wait()
    out = h8 + jnp.dot(act[:, :SIDE], w2[:SIDE, :], preferred_element_type=f32)[0:8]
    tail = [[None] * (M // 128) for _ in range(B)]
    for cp, (o, s) in zip(cp_2, w2_chunks):
        cp.wait()
        if o < F - TAIL:
            out = out + jnp.dot(act[:, o:o + s], w2[o:o + s, :], preferred_element_type=f32)[0:8]
            continue
        for r in range(o, o + s, 16):
            a = [at_ref[b, r - (F - TAIL):r - (F - TAIL) + 16, :] for b in range(B)]
            for t in range(M // 128):
                w = w2[r:r + 16, t * 128:(t + 1) * 128].astype(f32)
                for b in range(B):
                    prod = w * a[b]
                    prod = prod[0:8] + prod[8:16]
                    tail[b][t] = prod if tail[b][t] is None else tail[b][t] + prod
    tail = [jnp.concatenate(tail[b], axis=1) for b in range(B)]
    tail = jnp.where(odd, tail[1] + pltpu.roll(tail[1], 1, 0), tail[0] + pltpu.roll(tail[0], 7, 0))
    tail = tail + pltpu.roll(tail, 2, 0)
    tail = tail + pltpu.roll(tail, 4, 0)
    out = out + tail
    ob[...] = out[0:B].astype(ob.dtype)
    cp_out.start()


def _kernel(*refs):
    ins, o_hbm, scratch, ob, osem = refs[:9], refs[9], refs[10:-2], refs[-2], refs[-1]
    _, ckv, wq, _, _, _, w1, _, _ = scratch[:9]
    nsem = (4 + wq.shape[0] // CW + 2 * (ckv.shape[2] // CW) + ckv.shape[0] * (ckv.shape[1] // CK)
            + wq.shape[1] // CO + wq.shape[0] // C1 + len(_w2_chunks(w1.shape[1])))
    cp_out = pltpu.make_async_copy(ob, o_hbm, osem)
    pl.run_scoped(lambda sems: _body(*ins, *scratch, ob, cp_out, sems), pltpu.SemaphoreType.DMA((nsem,)))
    cp_out.wait()


@jax.jit
def pallas_sequential_preLN__compressed_kv_cla__dense_activation_mish__decode_kernel(
    A_x: jax.Array,
    A_c_kv: jax.Array,
    A_w_q: jax.Array,
    A_w_uk: jax.Array,
    A_w_uv: jax.Array,
    A_w_o: jax.Array,
    B_x: jax.Array,
    B_w1: jax.Array,
    B_b1: jax.Array,
    B_w2: jax.Array,
):
    del B_x
    B, Sq, M = A_x.shape
    _, H, D = A_w_q.shape
    DC = A_c_kv.shape[2]
    assert (B, Sq, H, D) == (2, 1, 32, 128), "the row packing assumes 2 batch entries, 1 query and 32 heads of 128"
    ins = (A_x.reshape(B, M), A_c_kv, A_w_q, A_w_uk, A_w_uv, A_w_o, B_w1, B_b1, B_w2)
    hbm = pl.BlockSpec(memory_space=pltpu.HBM)
    out = pl.pallas_call(
        _kernel,
        out_shape=jax.ShapeDtypeStruct((B, M), A_x.dtype),
        in_specs=[hbm] * len(ins),
        out_specs=hbm,
        scratch_shapes=[pltpu.VMEM(a.shape, a.dtype) for a in ins] + [
            pltpu.VMEM((CW // 2, CW * H), u32),
            pltpu.VMEM((M // CW * 8, CW * H), u32),
            pltpu.VMEM((B, DC // CW, H, CW), bf16),
            pltpu.VMEM((B, H, DC), f32),
            pltpu.SMEM((SIDE, M), B_w2.dtype),
            pltpu.VMEM((B, TAIL, 128), f32),
            pltpu.VMEM((B, M), A_x.dtype),
            pltpu.SemaphoreType.DMA(()),
        ],
        compiler_params=pltpu.CompilerParams(vmem_limit_bytes=64 * 1024 * 1024),
    )(*ins)
    return out.reshape(A_x.shape)
```
